```python
import jax
import jax.numpy as jnp

def _softmax(x, axis=-1):
    return jax.nn.softmax(x, axis=axis)
def _gelu(x):
    return jax.nn.gelu(x, approximate=True)
def _silu(x):
    return jax.nn.silu(x)
def _sigmoid(x):
    return jax.nn.sigmoid(x)
def _layernorm(x, axis=-1, eps=1e-5):
    m = jnp.mean(x, axis=axis, keepdims=True)
    v = jnp.var(x, axis=axis, keepdims=True)
    return (x - m) / jnp.sqrt(v + eps)
def _scatter_add(tgt, idx, src, axis=0):
    return tgt.at[idx].add(src)
def _segment_sum(src, seg, n):
    return jax.ops.segment_sum(src, seg, n)
class _Rng:
    def __init__(self, key):
        self._k = key
    def _next(self):
        self._k, sub = jax.random.split(self._k)
        return sub
    def normal(self, shape):
        return jax.random.normal(self._next(), shape, dtype=jnp.bfloat16)
    def randint(self, lo, hi, shape):
        return jax.random.randint(self._next(), shape, lo, hi, dtype=jnp.int32)
    def uniform(self, shape, lo=0.0, hi=1.0):
        return jax.random.uniform(self._next(), shape, jnp.bfloat16, lo, hi)
    def permutation(self, n):
        return jax.random.permutation(self._next(), n)


kernel_name = 'recurrent_scan__linear_kernel_hedgehog__dense_activation_relu__prompt'

def _fwd_setup_inputs():
    _rng = _Rng(jax.random.key(int.from_bytes(__import__("os").urandom(4), "little")))
    _w = (lambda a: (lambda t: t.astype(jnp.bfloat16) if jnp.issubdtype(t.dtype, jnp.floating) else t)(jnp.asarray(a)))
    def _A_setup():
        B, S, D, H = 1, 2048, 1024, 32
        Dh = D // H
        return {
            "x": _w((lambda *s: _rng.normal(s) * 0.05)(B, S, D)),
            "wqkv": _w((lambda *s: _rng.normal(s) * 0.05)(D, 3 * D)),
            "w_phi": _w((lambda *s: _rng.normal(s) * 0.05)(H, Dh, Dh) * (Dh ** -0.5)),
            "wo": _w((lambda *s: _rng.normal(s) * 0.05)(D, D)),
        }
    _A_in = _A_setup()

    def _B_setup():
        B, S, D, Dff = 1, 2048, 1024, 3584
        return {
            "x": _w((lambda *s: _rng.normal(s) * 0.05)(B, S, D)),
            "w1": _w((lambda *s: _rng.normal(s) * 0.05)(D, Dff)),
            "w2": _w((lambda *s: _rng.normal(s) * 0.05)(Dff, D)),
        }
    _B_in = _B_setup()

    return {
        "A_x": _A_in["x"],
        "A_wqkv": _A_in["wqkv"],
        "A_w_phi": _A_in["w_phi"],
        "A_wo": _A_in["wo"],
        "B_x": _B_in["x"],
        "B_w1": _B_in["w1"],
        "B_w2": _B_in["w2"],
    }

def _fwd_reference(A_x, A_wqkv, A_w_phi, A_wo, B_x, B_w1, B_w2):
    def _A_ref(x, wqkv, w_phi, wo):
        B, S, D = x.shape
        H = 32; Dh = D // H
        qkv = (lambda x, *d: x.transpose(*d))((x @ wqkv).reshape(B, S, 3, H, Dh), 2, 0, 3, 1, 4)
        q, k, v = qkv[0], qkv[1], qkv[2]
        pq = jnp.einsum("bhsd,hdf->bhsf", q, w_phi)
        pk = jnp.einsum("bhsd,hdf->bhsf", k, w_phi)
        phi_q = jnp.concatenate([_softmax(pq, axis=-1), _softmax(-pq, axis=-1)], axis=-1)
        phi_k = jnp.concatenate([_softmax(pk, axis=-1), _softmax(-pk, axis=-1)], axis=-1)
        kv = jnp.einsum("bhsf,bhsd->bhfd", phi_k, v)
        z  = jnp.einsum("bhsf->bhf", phi_k)
        num = jnp.einsum("bhqf,bhfd->bhqd", phi_q, kv)
        den = jnp.einsum("bhqf,bhf->bhq", phi_q, z)[..., None] + 1e-6
        o = num / den
        return (lambda x, *d: x.transpose(*d))(o, 0, 2, 1, 3).reshape(B, S, D) @ wo

    def _B_ref(x, w1, w2):
        h = jnp.einsum("bsd,df->bsf", x, w1)
        zero = jnp.zeros_like(h)
        h = jnp.maximum(h, zero)
        return jnp.einsum("bsf,fd->bsd", h, w2)

    x = A_x
    xn = _layernorm(x, axis=-1)
    s = _A_ref(xn, A_wqkv, A_w_phi, A_wo)
    g = _silu(_B_ref(xn, B_w1, B_w2))
    return x + s * g


def setup_inputs():
    _inp = _fwd_setup_inputs()
    _gk = jax.random.fold_in(jax.random.key(int.from_bytes(__import__("os").urandom(4), "little")), 2**31 - 1)
    _shapes = [[1, 2048, 1024]]
    _dtypes = ['bfloat16']
    _gks = jax.random.split(_gk, len(_shapes))
    _gs = [jax.random.normal(k, s, dtype=jnp.dtype(d)) * 0.05 for k, s, d in zip(_gks, _shapes, _dtypes)]
    _inp["grad_out"] = _gs[0]
    return _inp

def reference(A_x, A_wqkv, A_w_phi, A_wo, B_w1, B_w2, B_x, grad_out):
    _const = dict(B_x=B_x)
    def _f(*_d):
        return _fwd_reference(**{'A_x': _d[0], 'A_wqkv': _d[1], 'A_w_phi': _d[2], 'A_wo': _d[3], 'B_w1': _d[4], 'B_w2': _d[5], **_const})
    _out, _vjp = jax.vjp(_f, A_x, A_wqkv, A_w_phi, A_wo, B_w1, B_w2)
    _grads = _vjp(grad_out)
    _out0 = jnp.asarray(_out)
    return (_out0, *[jnp.asarray(_g) for _g in _grads])
```

```python
import jax
import jax.numpy as jnp
import jax.experimental.pallas as pl
import jax.experimental.pallas.tpu as pltpu

S = 2048
D = 1024
H = 32
DH = 32
DFF = 3584
NG = 8
T = 256
NT = S // T
EXT = 144

f32 = jnp.float32
bf16 = jnp.bfloat16


def _nn(a, b):
    return jnp.dot(a, b, preferred_element_type=f32)


def _nt(a, b):
    return jax.lax.dot_general(a, b, (((1,), (1,)), ((), ())), preferred_element_type=f32)


def _tn(a, b):
    return jax.lax.dot_general(a, b, (((0,), (0,)), ((), ())), preferred_element_type=f32)


def _iota(shape, dim):
    return jax.lax.broadcasted_iota(jnp.int32, shape, dim)


def _pair(v, op):
    return op(v, pltpu.roll(v, 4, v.ndim - 2))


def _phi(p):
    p4 = p.reshape(NG, 16, 8, p.shape[-1])
    mx = _pair(jnp.max(p4, axis=1), jnp.maximum)
    mn = _pair(jnp.min(p4, axis=1), jnp.minimum)
    ep = jnp.exp(p4 - mx[:, None])
    en = jnp.exp(mn[:, None] - p4)
    sp = _pair(jnp.sum(ep, axis=1), jnp.add)
    sn = _pair(jnp.sum(en, axis=1), jnp.add)
    return ep * (1.0 / sp)[:, None], en * (1.0 / sn)[:, None]


def _softmax_bwd(ph, dph):
    t = ph.shape[-1]
    ph = ph.reshape(2, 16, 8, t)
    dph = dph.reshape(2, 16, 8, t)
    u = ph * dph
    r = _pair(jnp.sum(u, axis=1), jnp.add)
    w = u - ph * r[:, None]
    return (w[0] - w[1]).reshape(128, t)


def _kernel(x_hbm, wqkv_hbm, wphi_ref, wo_hbm, w1_hbm, w2_hbm, do_hbm,
            out_hbm, dx_hbm, dwqkv_hbm, dwphi_ref, dwo_hbm, dw1_hbm, dw2_hbm,
            X, DO, WQKV, WO, W1, W2, WT, PHIPT, XN, RSTD, PHIQ, PHIK, VT, Hs, DHs, F, DS, OT,
            KVT, KVTm, KVm, ZB, DNE,
            isem, osem):
    cp_x = pltpu.make_async_copy(x_hbm, X, isem.at[0])
    cp_wqkv = pltpu.make_async_copy(wqkv_hbm, WQKV, isem.at[1])
    cp_wo = pltpu.make_async_copy(wo_hbm, WO, isem.at[2])
    cp_w1 = pltpu.make_async_copy(w1_hbm, W1, isem.at[3])
    cp_w2 = pltpu.make_async_copy(w2_hbm, W2, isem.at[4])
    cp_do = pltpu.make_async_copy(do_hbm, DO, isem.at[5])
    cp_wqkv.start()
    cp_x.start()
    cp_w1.start()
    cp_w2.start()
    cp_wo.start()
    cp_do.start()

    r128 = _iota((128, 128), 0)
    c128 = _iota((128, 128), 1)
    perm = jnp.where((r128 // 4 == c128 % 32) & (r128 % 4 == c128 // 32), 1.0, 0.0).astype(bf16)
    permT = jnp.where((c128 // 4 == r128 % 32) & (c128 % 4 == r128 // 32), 1.0, 0.0).astype(bf16)
    maskE = (_iota((EXT, 256), 0) % 4) == (_iota((EXT, 256), 1) % 4)

    E = jnp.where(_iota((32, 128), 1) // 4 == _iota((32, 128), 0), 1.0, 0.0).astype(bf16)
    rep = _nn(wphi_ref[...], E)
    phip = jnp.where((_iota((1024, 128), 0) // 32) % 4 == _iota((1024, 128), 1) % 4, rep, 0.0)
    for g in range(NG):
        PHIPT[g] = phip[g * 128:(g + 1) * 128, :].T.astype(bf16)

    VT[:, 128:EXT, :] = jnp.ones((NG, EXT - 128, S), bf16)
    KVT[...] = jnp.zeros_like(KVT)

    cp_wqkv.wait()
    for g in range(NG):
        WT[g * 128:(g + 1) * 128, :] = _nt(PHIPT[g], WQKV[:, g * 128:(g + 1) * 128]).astype(bf16)
        WT[D + g * 128:D + (g + 1) * 128, :] = _nt(PHIPT[g], WQKV[:, D + g * 128:D + (g + 1) * 128]).astype(bf16)
        WT[2 * D + g * 128:2 * D + (g + 1) * 128, :] = _nt(perm, WQKV[:, 2 * D + g * 128:2 * D + (g + 1) * 128]).astype(bf16)

    cp_x.wait()
    cp_w1.wait()
    cp_w2.wait()

    def phase_a(t, c):
        ts = pl.multiple_of(t * T, T)
        rows = pl.ds(ts, T)
        x = X[rows, :].astype(f32)
        mu = jnp.mean(x, axis=-1, keepdims=True)
        xc = x - mu
        var = jnp.mean(xc * xc, axis=-1, keepdims=True)
        rstd = jax.lax.rsqrt(var + 1e-5)
        xn = (xc * rstd).astype(bf16)
        XN[rows, :] = xn
        RSTD[rows, :] = jnp.broadcast_to(rstd, (T, 128))
        pT = _nt(WT[...], xn)
        VT[:, 0:128, rows] = pT[2 * D:3 * D].reshape(NG, 128, T).astype(bf16)
        kp, kn = _phi(pT[D:2 * D])
        PHIK[:, 0:128, rows] = kp.reshape(NG, 128, T).astype(bf16)
        PHIK[:, 128:256, rows] = kn.reshape(NG, 128, T).astype(bf16)
        qp, qn = _phi(pT[0:D])
        PHIQ[:, 0:128, rows] = qp.reshape(NG, 128, T).astype(bf16)
        PHIQ[:, 128:256, rows] = qn.reshape(NG, 128, T).astype(bf16)
        for g in range(NG):
            KVT[g] += _nt(VT[g, :, rows], PHIK[g, :, rows])
        h = jnp.maximum(_nn(xn, W1[...]), 0.0).astype(bf16)
        Hs[rows, :] = h
        F[rows, :] = _nn(h, W2[...]).astype(F.dtype)
        return c

    jax.lax.fori_loop(0, NT, phase_a, 0)

    def prep(col_from_masked):
        for g in range(NG):
            kvt = KVT[g]
            m = jnp.where(maskE, kvt, 0.0)
            KVTm[g] = m.astype(bf16)
            KVm[g] = m[0:128, :].T.astype(bf16)
            if col_from_masked:
                zrow = jnp.sum(m[128:132, :], axis=0, keepdims=True)
            else:
                zrow = kvt[128:129, :]
            ZB[g] = jnp.broadcast_to(zrow, (128, 256)).T

    prep(False)
    KVT[...] = jnp.zeros_like(KVT)

    cp_wo.wait()
    for g in range(NG):
        WO[g * 128:(g + 1) * 128, :] = _nn(perm, WO[g * 128:(g + 1) * 128, :]).astype(bf16)
    cp_do.wait()

    def out_copy(t):
        rows = pl.ds(pl.multiple_of(t * T, T), T)
        return pltpu.make_async_copy(X.at[rows, :], out_hbm.at[rows, :], osem.at[0])

    def dx_copy(t):
        rows = pl.ds(pl.multiple_of(t * T, T), T)
        return pltpu.make_async_copy(DO.at[rows, :], dx_hbm.at[rows, :], osem.at[1])

    def phase_b(t, c):
        ts = pl.multiple_of(t * T, T)
        rows = pl.ds(ts, T)
        o_l, rden_l = [], []
        for g in range(NG):
            ne = _nn(KVTm[g], PHIQ[g, :, rows])
            rden = 1.0 / (ne[128:136] + 1e-6)
            o_l.append(ne[0:128].reshape(16, 8, T) * rden[None])
            rden_l.append(rden)
        oT = jnp.concatenate([o.reshape(128, T) for o in o_l], axis=0).astype(bf16)
        OT[:, rows] = oT
        s = _tn(oT, WO[...])
        f = F[rows, :].astype(f32)
        sig = jax.nn.sigmoid(f)
        gate = f * sig
        dout = DO[rows, :].astype(f32)
        X[rows, :] = (X[rows, :].astype(f32) + s * gate).astype(bf16)
        out_copy(t).start()
        ds = (dout * gate).astype(bf16)
        DS[rows, :] = ds
        df = (dout * s * (sig * (1.0 + f * (1.0 - sig)))).astype(bf16)
        F[rows, :] = df
        doT = _nt(WO[...], ds)
        for g in range(NG):
            dnum = doT[g * 128:(g + 1) * 128].reshape(16, 8, T) * rden_l[g][None]
            dden = -_pair(jnp.sum(dnum * o_l[g], axis=0), jnp.add)
            dnb = dnum.reshape(128, T).astype(bf16)
            DNE[0:128, :] = dnb
            DNE[128:EXT, :] = jnp.concatenate([dden, dden], axis=0).astype(bf16)
            phq = PHIQ[g, :, rows]
            KVT[g] += _nt(DNE[...], phq)
            zb = ZB[g]
            zt = jnp.concatenate([zb] * (T // 128), axis=1).reshape(32, 8, T)
            dphi = _nn(KVm[g], dnb).reshape(32, 8, T) + zt * dden[None]
            dp = _softmax_bwd(phq.astype(f32), dphi.reshape(256, T))
            PHIQ[g, 0:128, rows] = dp.astype(bf16)
        dh = _nt(df, W2[...])
        DHs[rows, :] = jnp.where(Hs[rows, :] > 0, dh, 0.0).astype(bf16)
        return c

    jax.lax.fori_loop(0, NT, phase_b, 0)

    prep(True)

    CH = 512
    def dw2_copy(i):
        rows = pl.ds(pl.multiple_of(i * CH, CH), CH)
        return pltpu.make_async_copy(W2.at[rows, :], dw2_hbm.at[rows, :], osem.at[2])

    def dw2_body(i, c):
        cs = pl.multiple_of(i * CH, CH)
        W2[pl.ds(cs, CH), :] = _tn(Hs[:, pl.ds(cs, CH)], F[...]).astype(bf16)
        dw2_copy(i).start()
        return c

    jax.lax.fori_loop(0, DFF // CH, dw2_body, 0)

    for half in range(2):
        r0 = half * 512
        dwop = _nn(OT[r0:r0 + 512, :], DS[...]).astype(bf16)
        for gg in range(4):
            WO[r0 + gg * 128:r0 + (gg + 1) * 128, :] = _nn(permT, dwop[gg * 128:(gg + 1) * 128, :]).astype(bf16)
    cp_dwo = pltpu.make_async_copy(WO, dwo_hbm, osem.at[3])
    cp_dwo.start()

    def phase_c(t, c):
        ts = pl.multiple_of(t * T, T)
        rows = pl.ds(ts, T)
        for g in range(NG):
            phk = PHIK[g, :, rows]
            zb = ZB[g]
            zt = jnp.concatenate([zb] * (T // 128), axis=1)
            dphi = _nn(KVm[g], VT[g, 0:128, rows]) + zt
            dv = _nn(KVTm[g, 0:128, :], phk)
            dp = _softmax_bwd(phk.astype(f32), dphi)
            PHIK[g, 0:128, rows] = dp.astype(bf16)
            VT[g, 0:128, rows] = dv.astype(bf16)
        dxn = _nt(DHs[rows, :], W1[...])
        dxn += _tn(PHIQ[:, 0:128, rows].reshape(D, T), WT[0:D, :])
        dxn += _tn(PHIK[:, 0:128, rows].reshape(D, T), WT[D:2 * D, :])
        dxn += _tn(VT[:, 0:128, rows].reshape(D, T), WT[2 * D:3 * D, :])
        xn = XN[rows, :].astype(f32)
        rstd = RSTD[rows, 0:1]
        m1 = jnp.mean(dxn, axis=-1, keepdims=True)
        m2 = jnp.mean(dxn * xn, axis=-1, keepdims=True)
        DO[rows, :] = (DO[rows, :].astype(f32) + rstd * (dxn - m1 - xn * m2)).astype(bf16)
        dx_copy(t).start()
        return c

    jax.lax.fori_loop(0, NT, phase_c, 0)

    def dw1_copy(i):
        cols = pl.ds(pl.multiple_of(i * CH, CH), CH)
        return pltpu.make_async_copy(W1.at[:, cols], dw1_hbm.at[:, cols], osem.at[4])

    def dw1_body(i, c):
        cs = pl.multiple_of(i * CH, CH)
        W1[:, pl.ds(cs, CH)] = _tn(XN[...], DHs[:, pl.ds(cs, CH)]).astype(bf16)
        dw1_copy(i).start()
        return c

    jax.lax.fori_loop(0, DFF // CH, dw1_body, 0)

    ET = jnp.where(_iota((128, 32), 0) // 4 == _iota((128, 32), 1), 1.0, 0.0).astype(bf16)
    maskP = (r128 % 4) == (c128 // 32)

    def dwqkv_copy(i):
        cols = pl.ds(i * 512, 512)
        return pltpu.make_async_copy(WQKV.at[:, cols], dwqkv_hbm.at[:, cols], osem.at[5])

    for half in range(2):
        gt = _nn(VT[half * 4:(half + 1) * 4, 0:128, :].reshape(512, S), XN[...]).astype(bf16)
        for gg in range(4):
            g = half * 4 + gg
            WQKV[:, 2 * D + g * 128:2 * D + (g + 1) * 128] = _tn(gt[gg * 128:(gg + 1) * 128, :], perm).astype(bf16)
        dwqkv_copy(4 + half).start()
    for half in range(2):
        gq = _nn(PHIQ[half * 4:(half + 1) * 4, 0:128, :].reshape(512, S), XN[...]).astype(bf16)
        gk = _nn(PHIK[half * 4:(half + 1) * 4, 0:128, :].reshape(512, S), XN[...]).astype(bf16)
        for gg in range(4):
            g = half * 4 + gg
            gq_g = gq[gg * 128:(gg + 1) * 128, :]
            gk_g = gk[gg * 128:(gg + 1) * 128, :]
            dpt = _nn(gq_g, WQKV[:, g * 128:(g + 1) * 128]) + _nn(gk_g, WQKV[:, D + g * 128:D + (g + 1) * 128])
            dpt = jnp.where(maskP, dpt, 0.0).astype(bf16)
            dwphi_ref[g * 128:(g + 1) * 128, :] = _tn(dpt, ET).astype(bf16)
            WQKV[:, g * 128:(g + 1) * 128] = _tn(gq_g, PHIPT[g]).astype(bf16)
            WQKV[:, D + g * 128:D + (g + 1) * 128] = _tn(gk_g, PHIPT[g]).astype(bf16)
        dwqkv_copy(half).start()
        dwqkv_copy(2 + half).start()

    pltpu.make_async_copy(X, out_hbm, osem.at[0]).wait()
    pltpu.make_async_copy(DO, dx_hbm, osem.at[1]).wait()
    pltpu.make_async_copy(W2, dw2_hbm, osem.at[2]).wait()
    cp_dwo.wait()
    pltpu.make_async_copy(W1, dw1_hbm, osem.at[4]).wait()
    pltpu.make_async_copy(WQKV, dwqkv_hbm, osem.at[5]).wait()


@jax.jit
def pallas_recurrent_scan__linear_kernel_hedgehog__dense_activation_relu__prompt_kernel(
    A_x: jax.Array,
    A_wqkv: jax.Array,
    A_w_phi: jax.Array,
    A_wo: jax.Array,
    B_x: jax.Array,
    B_w1: jax.Array,
    B_w2: jax.Array,
    grad_out: jax.Array,
):
    x2 = A_x.reshape(S, D)
    do2 = grad_out.reshape(S, D)
    wphi2 = A_w_phi.reshape(H * DH, DH)
    anyspec = pl.BlockSpec(memory_space=pl.ANY)
    vspec = pl.BlockSpec(memory_space=pltpu.VMEM)
    out_shape = (
        jax.ShapeDtypeStruct((S, D), bf16),
        jax.ShapeDtypeStruct((S, D), bf16),
        jax.ShapeDtypeStruct((D, 3 * D), bf16),
        jax.ShapeDtypeStruct((H * DH, DH), bf16),
        jax.ShapeDtypeStruct((D, D), bf16),
        jax.ShapeDtypeStruct((D, DFF), bf16),
        jax.ShapeDtypeStruct((DFF, D), bf16),
    )
    scratch = [
        pltpu.VMEM((S, D), bf16),
        pltpu.VMEM((S, D), bf16),
        pltpu.VMEM((D, 3 * D), bf16),
        pltpu.VMEM((D, D), bf16),
        pltpu.VMEM((D, DFF), bf16),
        pltpu.VMEM((DFF, D), bf16),
        pltpu.VMEM((3 * D, D), bf16),
        pltpu.VMEM((NG, 128, 128), bf16),
        pltpu.VMEM((S, D), bf16),
        pltpu.VMEM((S, 128), f32),
        pltpu.VMEM((NG, 256, S), bf16),
        pltpu.VMEM((NG, 256, S), bf16),
        pltpu.VMEM((NG, EXT, S), bf16),
        pltpu.VMEM((S, DFF), bf16),
        pltpu.VMEM((S, DFF), bf16),
        pltpu.VMEM((S, D), bf16),
        pltpu.VMEM((S, D), bf16),
        pltpu.VMEM((D, S), bf16),
        pltpu.VMEM((NG, EXT, 256), f32),
        pltpu.VMEM((NG, EXT, 256), bf16),
        pltpu.VMEM((NG, 256, 128), bf16),
        pltpu.VMEM((NG, 256, 128), f32),
        pltpu.VMEM((EXT, T), bf16),
        pltpu.SemaphoreType.DMA((6,)),
        pltpu.SemaphoreType.DMA((6,)),
    ]
    outs = pl.pallas_call(
        _kernel,
        out_shape=out_shape,
        in_specs=[anyspec, anyspec, vspec, anyspec, anyspec, anyspec, anyspec],
        out_specs=(anyspec, anyspec, anyspec, vspec, anyspec, anyspec, anyspec),
        scratch_shapes=scratch,
        compiler_params=pltpu.CompilerParams(vmem_limit_bytes=127 * 2**20),
    )(x2, A_wqkv, wphi2, A_wo, B_w1, B_w2, do2)
    out, dx, dwqkv, dwphi, dwo, dw1, dw2 = outs
    return (out.reshape(1, S, D), dx.reshape(1, S, D), dwqkv, dwphi.reshape(H, DH, DH), dwo, dw1, dw2)
```

```python
import jax
import jax.numpy as jnp
import jax.experimental.pallas as pl
import jax.experimental.pallas.tpu as pltpu

S = 2048
D = 1024
H = 32
DH = 32
DFF = 3584
NB = 8
NG = 16
T = 256
NT = S // T
EXT = 80
CH = 512
NCH = DFF // CH
XT = 256
NXT = S // XT
FR = 208
LB = 8
LF = 16

f32 = jnp.float32
bf16 = jnp.bfloat16


def _nn(a, b):
    return jnp.dot(a, b, preferred_element_type=f32)


def _nt(a, b):
    return jax.lax.dot_general(a, b, (((1,), (1,)), ((), ())), preferred_element_type=f32)


def _tn(a, b):
    return jax.lax.dot_general(a, b, (((0,), (0,)), ((), ())), preferred_element_type=f32)


def _iota(shape, dim):
    return jax.lax.broadcasted_iota(jnp.int32, shape, dim)


def _zero_after(v):
    return jnp.where(v * v < 0.0, 1.0, 0.0)


def _pair(v, op):
    v = op(v, pltpu.roll(v, 4, v.ndim - 2))
    return op(v, pltpu.roll(v, 2, v.ndim - 2))


def _phi(p):
    p4 = p.reshape(NG, 8, 8, p.shape[-1])
    mx = _pair(jnp.max(p4, axis=1), jnp.maximum)
    mn = _pair(jnp.min(p4, axis=1), jnp.minimum)
    ep = jnp.exp(p4 - mx[:, None])
    en = jnp.exp(mn[:, None] - p4)
    sp = _pair(jnp.sum(ep, axis=1), jnp.add)
    sn = _pair(jnp.sum(en, axis=1), jnp.add)
    return ep * (1.0 / sp)[:, None], en * (1.0 / sn)[:, None]


def _softmax_bwd(ph, dph):
    t = ph.shape[-1]
    ph = ph.reshape(2, 8, 8, t)
    dph = dph.reshape(2, 8, 8, t)
    u = ph * dph
    r = _pair(jnp.sum(u, axis=1), jnp.add)
    w = u - ph * r[:, None]
    return (w[0] - w[1]).reshape(64, t)


def _kernel(x_hbm, wqkv_hbm, wphi_hbm, wo_hbm, w1_hbm, w2_hbm, do_hbm,
            out_hbm, dx_hbm, dwqkv_hbm, dwphi_hbm, dwo_hbm, dw1_hbm, dw2_hbm,
            X, DO, WQKV, WO, W1, W2, WT, PHIPT, XN, RSTD, PHIQ, PHIK, VT, Hs, DHs, F, DS, OT,
            KVT, KVTm, KVm, ZB, DNE, DXN, wphi_ref,
            xsem, wsem, isem, osem, qsem):
    XB = (0, 512, 896, 2048)

    def cp_x(i):
        return pltpu.make_async_copy(x_hbm.at[XB[i]:XB[i + 1], :], X.at[XB[i]:XB[i + 1], :], xsem.at[i])

    def cp_w1(i):
        return pltpu.make_async_copy(w1_hbm.at[:, i * CH:(i + 1) * CH], W1.at[:, i * CH:(i + 1) * CH], wsem.at[i])

    def cp_wqkv(i, part):
        cols = pl.ds(pl.multiple_of(part * D + i * 256, 256), 256)
        return pltpu.make_async_copy(wqkv_hbm.at[:, cols], WQKV.at[:, cols], qsem.at[3 * i + part])

    cp_wo = pltpu.make_async_copy(wo_hbm, WO, isem.at[1])
    cp_w2 = pltpu.make_async_copy(w2_hbm, W2, isem.at[2])
    cp_do = pltpu.make_async_copy(do_hbm, DO, isem.at[3])
    cp_wphi = pltpu.make_async_copy(wphi_hbm, wphi_ref, isem.at[4])
    dwphi_ref = wphi_ref
    cp_x(0).start()
    cp_w1(0).start()

    r128 = _iota((128, 128), 0)
    c128 = _iota((128, 128), 1)
    def head_of(r):
        return (r // 64) * 2 + r % 2

    def feat_of(r):
        return (r % 64) // 2

    rE = _iota((EXT, 128), 0)
    maskE = jnp.where(rE < 64, rE // 32, (rE - 64) // 8) == (_iota((EXT, 128), 1) % 2)

    VT[:, 64:EXT, :] = jnp.ones((NG, EXT - 64, S), bf16)
    KVT[...] = jnp.zeros_like(KVT)
    KVm[...] = jnp.zeros_like(KVm)

    def ln_fwd(r0, n, chain):
        dep = None
        for a in range(0, n, LF):
            rows = pl.ds(pl.multiple_of(r0 + a, LF), LF)
            x = X[rows, :].astype(f32)
            mu = jnp.mean(x, axis=-1, keepdims=True)
            if chain and dep is not None:
                mu = mu + _zero_after(dep)
            xc = x - mu
            var = jnp.mean(xc * xc, axis=-1, keepdims=True)
            rstd = jax.lax.rsqrt(var + 1e-5)
            dep = rstd
            XN[rows, :] = (xc * rstd).astype(bf16)
            RSTD[rows, :] = jnp.broadcast_to(rstd, (LF, 128))

    def h_mm(r0, r1, j):
        Hs[r0:r1, j * CH:(j + 1) * CH] = jnp.maximum(_nn(XN[r0:r1, :], W1[:, j * CH:(j + 1) * CH]), 0.0).astype(bf16)

    R0 = XB[1]
    RB = 384
    NRB = (S - R0) // RB
    with jax.named_scope("s1a"):
        cp_x(0).wait()
        cp_w1(1).start()
        cp_w1(2).start()
        ln_fwd(0, R0, False)
        cp_w1(0).wait()
        for j in range(3, NCH):
            cp_w1(j).start()
        h_mm(0, R0, 0)
        cp_w1(1).wait()
        cp_w1(2).wait()
        cp_wphi.start()
        h_mm(0, R0, 1)
        h_mm(0, R0, 2)
        for j in range(3, NCH):
            cp_w1(j).wait()
        cp_x(1).start()
        cp_x(2).start()
        h_mm(0, R0, 3)
        h_mm(0, R0, 4)
        cp_x(1).wait()
        cp_wphi.wait()
        for i in range(4):
            for part in range(3):
                cp_wqkv(i, part).start()
        E = jnp.where(feat_of(_iota((32, 128), 1)) == _iota((32, 128), 0), 1.0, 0.0).astype(bf16)
        rep = _nn(wphi_ref[...], E)
        phip = jnp.where((_iota((1024, 128), 0) // 32) % 4 == head_of(_iota((1024, 128), 1)), rep, 0.0)
        for g in range(NB):
            PHIPT[g] = phip[g * 128:(g + 1) * 128, :].T.astype(bf16)

        ln_fwd(R0, RB, True)
        h_mm(0, R0, 5)
        h_mm(0, R0, 6)

    def s1b_body(i, c):
        rows = pl.ds(pl.multiple_of(R0 + i * RB, 128), RB)
        xn = XN[rows, :]
        ln_fwd(R0 + jnp.minimum(i + 1, NRB - 1) * RB, RB, True)
        for j in range(NCH):
            Hs[rows, j * CH:(j + 1) * CH] = jnp.maximum(_nn(xn, W1[:, j * CH:(j + 1) * CH]), 0.0).astype(bf16)
            if j == 4:
                for part in range(3):
                    cp_wqkv(i, part).wait()
            if j in (4, 5):
                g = 2 * i + (j == 5)
                c0 = pl.multiple_of(g * 128, 128)
                pt = PHIPT[g]
                WT[pl.ds(c0, 128), :] = _nt(pt, WQKV[:, pl.ds(c0, 128)]).astype(bf16)
                WT[pl.ds(D + c0, 128), :] = _nt(pt, WQKV[:, pl.ds(D + c0, 128)]).astype(bf16)
                WT[pl.ds(2 * D + c0, 128), :] = WQKV[:, pl.ds(2 * D + c0, 128)].T
        return c

    with jax.named_scope("s1b"):
        cp_x(2).wait()
        cp_w2.start()
        cp_wo.start()
        cp_do.start()
        jax.lax.fori_loop(0, (S - R0) // RB, s1b_body, 0)
        cp_w2.wait()
        cp_wo.wait()
        cp_do.wait()

    def phase_a(t, c):
        ts = pl.multiple_of(t * T, T)
        rows = pl.ds(ts, T)
        xn = XN[rows, :]
        kp, kn = _phi(_nt(WT[D:2 * D, :], xn))
        PHIK[:, 0:64, rows] = kp.reshape(NG, 64, T).astype(bf16)
        PHIK[:, 64:128, rows] = kn.reshape(NG, 64, T).astype(bf16)
        VT[:, 0:64, rows] = _nt(WT[2 * D:3 * D, :], xn).reshape(NG, 64, T).astype(bf16)
        qp, qn = _phi(_nt(WT[0:D, :], xn))
        PHIQ[:, 0:64, rows] = qp.reshape(NG, 64, T).astype(bf16)
        PHIQ[:, 64:128, rows] = qn.reshape(NG, 64, T).astype(bf16)
        for g in range(NG):
            KVT[g] += _nt(VT[g, :, rows], PHIK[g, :, rows])
        frows = pl.ds(pl.multiple_of(t * FR, 16), FR)
        F[frows, :] = _nn(Hs[frows, :], W2[...]).astype(F.dtype)
        return c

    with jax.named_scope("phaseA"):
        jax.lax.fori_loop(0, NT, phase_a, 0)

    def prep(col_from_masked):
        for p in range(NB):
            ms, zs = [], []
            for e in range(2):
                g = 2 * p + e
                kvt = KVT[g]
                m = jnp.where(maskE, kvt, 0.0)
                KVTm[g] = m.astype(bf16)
                ms.append(m[0:64, :])
                if col_from_masked:
                    zs.append(m[64:65, :] + m[72:73, :])
                else:
                    zs.append(kvt[64:65, :])
            mt = jnp.concatenate(ms, axis=0).T.astype(bf16)
            KVm[p, 0:128, 0:64] = mt[:, 0:64]
            KVm[p, 128:256, 64:128] = mt[:, 64:128]
            for e in range(2):
                ZB[2 * p + e] = jnp.broadcast_to(zs[e], (128, 128)).T

    def out_copy(t):
        rows = pl.ds(pl.multiple_of(t * T, T), T)
        return pltpu.make_async_copy(X.at[rows, :], out_hbm.at[rows, :], osem.at[0])

    def dx_copy(t):
        rows = pl.ds(pl.multiple_of(t * T, T), T)
        return pltpu.make_async_copy(DO.at[rows, :], dx_hbm.at[rows, :], osem.at[1])

    DC = 128
    NDC = DFF // DC

    def dh_mm(t, c0=0, c1=NDC, dfp=None):
        rows = pl.ds(pl.multiple_of(t * T, T), T)
        cols = slice(c0 * DC, c1 * DC)
        if dfp is None:
            dfp = F[rows, :]
        dh = _nt(dfp, W2[cols, :])
        DHs[rows, cols] = jnp.where(Hs[rows, cols] > 0, dh, 0.0).astype(bf16)

    def phase_b_main(t, filler):
        ts = pl.multiple_of(t * T, T)
        rows = pl.ds(ts, T)
        fc = [0]

        def fill(n):
            for _ in range(n):
                filler(fc[0])
                fc[0] += 1

        fill(2)
        o_l, rden_l = [], []
        odd = (_iota((8, T), 0) % 2) == 1
        for g in range(NG):
            ne = _nn(KVTm[g], PHIQ[g, :, rows])
            rden = (1.0 / (ne[64:80] + 1e-6)).reshape(2, 1, 8, T)
            o_l.append(ne[0:64].reshape(2, 4, 8, T) * rden)
            rden_l.append(rden)
            if g % 4 == 3:
                fill(1)
        f = F[rows, :].astype(f32)
        sig = jax.nn.sigmoid(f)
        gate = f * sig
        dout = DO[rows, :].astype(f32)
        ds = (dout * gate).astype(bf16)
        DS[rows, :] = ds
        fill(2)
        doT = _nt(WO[...], ds)
        oT = jnp.concatenate([o.reshape(64, T) for o in o_l], axis=0).astype(bf16)
        OT[:, rows] = oT
        s = _tn(oT, WO[...])
        X[rows, :] = (X[rows, :].astype(f32) + s * gate).astype(bf16)
        out_copy(t).start()
        df = (dout * s * (sig * (1.0 + f * (1.0 - sig)))).astype(bf16)
        F[rows, :] = df
        fill(2)
        for p in range(NB):
            ddens = []
            for e in range(2):
                g = 2 * p + e
                dnum = doT[g * 64:(g + 1) * 64].reshape(2, 4, 8, T) * rden_l[g]
                dd = jnp.sum(dnum * o_l[g], axis=1)
                dd = _pair(dd, jnp.add)
                dd = -(dd + pltpu.roll(dd, 1, 1))
                DNE[g, 0:64, :] = dnum.reshape(64, T).astype(bf16)
                DNE[g, 64:EXT, :] = dd.reshape(16, T).astype(bf16)
                ddens.append(jnp.where(odd, dd[1], dd[0]))
            dphi2 = _nn(KVm[p], DNE[2 * p:2 * p + 2, 0:64, :].reshape(128, T))
            for e in range(2):
                g = 2 * p + e
                phq = PHIQ[g, :, rows]
                KVT[g] += _nt(DNE[g], phq)
                zt = jnp.concatenate([ZB[g]] * (T // 128), axis=1).reshape(16, 8, T)
                dphi = dphi2[e * 128:(e + 1) * 128].reshape(16, 8, T) + zt * ddens[e][None]
                dp = _softmax_bwd(phq.astype(f32), dphi.reshape(128, T))
                PHIQ[g, 0:64, rows] = dp.astype(bf16)
            fill(2)
        fill(2)

    def phase_b(t, c):
        dfp = F[pl.ds(pl.multiple_of((t - 1) * T, T), T), :]
        phase_b_main(t, lambda i: dh_mm(t - 1, i, i + 1, dfp))
        return c

    def f_tail(i):
        if i < 8:
            cols = slice(i * 128, (i + 1) * 128)
            F[NT * FR:S, cols] = _nn(Hs[NT * FR:S, :], W2[:, cols]).astype(F.dtype)

    with jax.named_scope("prep1"):
        prep(False)
        KVT[...] = jnp.zeros_like(KVT)
        order = {0: 0, 3: 1, 6: 2, 8: 3, 12: 4, 16: 5, 20: 6, 24: 7}
        phase_b_main(0, lambda i: f_tail(order.get(i, 99)))

    with jax.named_scope("phaseB"):
        jax.lax.fori_loop(1, NT, phase_b, 0)

    with jax.named_scope("dh7"):
        prep(True)
        dh_mm(NT - 1)
        DXN[...] = jnp.zeros_like(DXN)

    def ln_bwd_rows(t, a0, n):
        dep = None
        for a in range(0, n, LB):
            rows = pl.ds(pl.multiple_of(t * T + a0 + a, LB), LB)
            dxn = DXN[pl.ds(pl.multiple_of(a0 + a, LB), LB), :]
            xn = XN[rows, :].astype(f32)
            rstd = RSTD[rows, 0:1]
            m1 = jnp.mean(dxn, axis=-1, keepdims=True)
            if dep is not None:
                m1 = m1 + _zero_after(dep)
            m2 = jnp.mean(dxn * xn, axis=-1, keepdims=True)
            r = rstd * (dxn - m1 - xn * m2)
            dep = r[:, 0:1]
            DO[rows, :] = (DO[rows, :].astype(f32) + r).astype(bf16)

    def phase_c_main(t):
        ts = pl.multiple_of(t * T, T)
        rows = pl.ds(ts, T)
        parts = []
        for p in range(NB):
            dphi2 = _nn(KVm[p], VT[2 * p:2 * p + 2, 0:64, rows].reshape(128, T))
            for e in range(2):
                g = 2 * p + e
                phk = PHIK[g, :, rows]
                zt = jnp.concatenate([ZB[g]] * (T // 128), axis=1)
                dphi = dphi2[e * 128:(e + 1) * 128] + zt
                dv = _nn(KVTm[g, 0:64, :], phk)
                dp = _softmax_bwd(phk.astype(f32), dphi)
                PHIK[g, 0:64, rows] = dp.astype(bf16)
                VT[g, 0:64, rows] = dv.astype(bf16)
            parts.append(_nt(DHs[rows, :], W1[p * 128:(p + 1) * 128, :]))
        dxn = jnp.concatenate(parts, axis=1)
        dxn += _tn(PHIQ[:, 0:64, rows].reshape(D, T), WT[0:D, :])
        dxn += _tn(PHIK[:, 0:64, rows].reshape(D, T), WT[D:2 * D, :])
        dxn += _tn(VT[:, 0:64, rows].reshape(D, T), WT[2 * D:3 * D, :])
        return dxn

    def phase_c(t, c):
        ln_bwd_rows(jnp.maximum(t - 1, 0), 0, T)
        DXN[...] = phase_c_main(t)

        @pl.when(t > 0)
        def _():
            dx_copy(t - 1).start()
        return c

    with jax.named_scope("phaseC"):
        jax.lax.fori_loop(0, NT, phase_c, 0)

    C2 = 896
    NC2 = DFF // C2

    def mid_body(i, c):
        r0 = pl.multiple_of(i * 256, 256)
        q0 = pl.multiple_of(i * 64, 64)
        ln_bwd_rows(NT - 1, q0, 64)
        lrows = pl.ds((NT - 1) * T + q0, 64)
        pltpu.make_async_copy(DO.at[lrows, :], dx_hbm.at[lrows, :], osem.at[1]).start()
        WO[pl.ds(r0, 256), :] = _nn(OT[pl.ds(r0, 256), :], DS[...]).astype(bf16)
        pltpu.make_async_copy(WO.at[pl.ds(r0, 256), :], dwo_hbm.at[pl.ds(r0, 256), :], osem.at[3]).start()
        cs = pl.multiple_of(i * C2, 128)
        W2[pl.ds(cs, C2), :] = _tn(Hs[:, pl.ds(cs, C2)], F[...]).astype(bf16)
        pltpu.make_async_copy(W2.at[pl.ds(cs, C2), :], dw2_hbm.at[pl.ds(cs, C2), :], osem.at[2]).start()
        OT[pl.ds(r0, 256), :] = XN[:, pl.ds(r0, 256)].T
        return c

    with jax.named_scope("dw2"):
        jax.lax.fori_loop(0, NC2, mid_body, 0)

    ET = jnp.where(feat_of(_iota((128, 32), 0)) == _iota((128, 32), 1), 1.0, 0.0).astype(bf16)
    maskP = head_of(r128) == (c128 // 32)

    def wq_copy(c0):
        cols = pl.ds(c0, 128)
        return pltpu.make_async_copy(WQKV.at[:, cols], dwqkv_hbm.at[:, cols], osem.at[5])

    def fin_body(i, c):
        def g_mm(ref):
            return _nn(ref[pl.ds(i * 2, 2), 0:64, :].reshape(128, S), XN[...]).astype(bf16)

        c0 = pl.multiple_of(i * 128, 128)
        rws = pl.ds(c0, 128)

        def dw1_mm(a, b):
            W1[rws, a:b] = _nn(OT[rws, :], DHs[:, a:b]).astype(bf16)

        gq = g_mm(PHIQ)
        gk = g_mm(PHIK)
        dw1_mm(0, 1024)
        cq = pl.ds(c0, 128)
        ck = pl.ds(D + c0, 128)
        dpt = _nn(gq, WQKV[:, cq]) + _nn(gk, WQKV[:, ck])
        dpt = jnp.where(maskP, dpt, 0.0).astype(bf16)
        pt = PHIPT[i]
        WQKV[:, cq] = _tn(gq, pt).astype(bf16)
        WQKV[:, ck] = _tn(gk, pt).astype(bf16)
        WQKV[:, pl.ds(2 * D + c0, 128)] = _nt(OT[...], VT[pl.ds(i * 2, 2), 0:64, :].reshape(128, S)).astype(bf16)
        dwphi_ref[rws, :] = _tn(dpt, ET).astype(bf16)
        pltpu.make_async_copy(wphi_ref.at[rws, :], dwphi_hbm.at[rws, :], osem.at[6]).start()
        wq_copy(c0).start()
        wq_copy(D + c0).start()
        wq_copy(2 * D + c0).start()
        dw1_mm(1024, 2560)
        pltpu.make_async_copy(W1.at[rws, 0:2560], dw1_hbm.at[rws, 0:2560], osem.at[4]).start()
        dw1_mm(2560, DFF)
        pltpu.make_async_copy(W1.at[rws, 2560:DFF], dw1_hbm.at[rws, 2560:DFF], osem.at[4]).start()
        return c

    with jax.named_scope("final"):
        jax.lax.fori_loop(0, NB, fin_body, 0)

    with jax.named_scope("drain"):
        pltpu.make_async_copy(X, out_hbm, osem.at[0]).wait()
        pltpu.make_async_copy(W2, dw2_hbm, osem.at[2]).wait()
        pltpu.make_async_copy(WO, dwo_hbm, osem.at[3]).wait()
        pltpu.make_async_copy(DO, dx_hbm, osem.at[1]).wait()
        pltpu.make_async_copy(WQKV, dwqkv_hbm, osem.at[5]).wait()
        pltpu.make_async_copy(W1, dw1_hbm, osem.at[4]).wait()
        pltpu.make_async_copy(wphi_ref, dwphi_hbm, osem.at[6]).wait()


@jax.jit
def pallas_recurrent_scan__linear_kernel_hedgehog__dense_activation_relu__prompt_kernel(
    A_x: jax.Array,
    A_wqkv: jax.Array,
    A_w_phi: jax.Array,
    A_wo: jax.Array,
    B_x: jax.Array,
    B_w1: jax.Array,
    B_w2: jax.Array,
    grad_out: jax.Array,
):
    x2 = A_x.reshape(S, D)
    do2 = grad_out.reshape(S, D)
    wphi2 = A_w_phi.reshape(H * DH, DH)
    anyspec = pl.BlockSpec(memory_space=pl.ANY)
    vspec = pl.BlockSpec(memory_space=pltpu.VMEM)
    out_shape = (
        jax.ShapeDtypeStruct((S, D), bf16),
        jax.ShapeDtypeStruct((S, D), bf16),
        jax.ShapeDtypeStruct((D, 3 * D), bf16),
        jax.ShapeDtypeStruct((H * DH, DH), bf16),
        jax.ShapeDtypeStruct((D, D), bf16),
        jax.ShapeDtypeStruct((D, DFF), bf16),
        jax.ShapeDtypeStruct((DFF, D), bf16),
    )
    scratch = [
        pltpu.VMEM((S, D), bf16),
        pltpu.VMEM((S, D), bf16),
        pltpu.VMEM((D, 3 * D), bf16),
        pltpu.VMEM((D, D), bf16),
        pltpu.VMEM((D, DFF), bf16),
        pltpu.VMEM((DFF, D), bf16),
        pltpu.VMEM((3 * D, D), bf16),
        pltpu.VMEM((NB, 128, 128), bf16),
        pltpu.VMEM((S, D), bf16),
        pltpu.VMEM((S, 128), f32),
        pltpu.VMEM((NG, 128, S), bf16),
        pltpu.VMEM((NG, 128, S), bf16),
        pltpu.VMEM((NG, EXT, S), bf16),
        pltpu.VMEM((S, DFF), bf16),
        pltpu.VMEM((S, DFF), bf16),
        pltpu.VMEM((S, D), bf16),
        pltpu.VMEM((S, D), bf16),
        pltpu.VMEM((D, S), bf16),
        pltpu.VMEM((NG, EXT, 128), f32),
        pltpu.VMEM((NG, EXT, 128), bf16),
        pltpu.VMEM((NB, 256, 128), bf16),
        pltpu.VMEM((NG, 128, 128), f32),
        pltpu.VMEM((NG, EXT, T), bf16),
        pltpu.VMEM((T, D), f32),
        pltpu.VMEM((H * DH, DH), bf16),
        pltpu.SemaphoreType.DMA((4,)),
        pltpu.SemaphoreType.DMA((NCH,)),
        pltpu.SemaphoreType.DMA((5,)),
        pltpu.SemaphoreType.DMA((7,)),
        pltpu.SemaphoreType.DMA((12,)),
    ]
    outs = pl.pallas_call(
        _kernel,
        out_shape=out_shape,
        in_specs=[anyspec] * 7,
        out_specs=(anyspec,) * 7,
        scratch_shapes=scratch,
        compiler_params=pltpu.CompilerParams(vmem_limit_bytes=127 * 2**20),
    )(x2, A_wqkv, wphi2, A_wo, B_w1, B_w2, do2)
    out, dx, dwqkv, dwphi, dwo, dw1, dw2 = outs
    return (out.reshape(1, S, D), dx.reshape(1, S, D), dwqkv, dwphi.reshape(H, DH, DH), dwo, dw1, dw2)
```

```python
import jax
import jax.numpy as jnp
import jax.experimental.pallas as pl
import jax.experimental.pallas.tpu as pltpu

S = 2048
D = 1024
H = 32
DH = 32
DFF = 3584
NB = 8
NG = 16
T = 256
NT = S // T
EXT = 80
CH = 512
NCH = DFF // CH
FR = 176
LB = 8
LF = 16

f32 = jnp.float32
bf16 = jnp.bfloat16


def _nn(a, b):
    return jnp.dot(a, b, preferred_element_type=f32)


def _nt(a, b):
    return jax.lax.dot_general(a, b, (((1,), (1,)), ((), ())), preferred_element_type=f32)


def _tn(a, b):
    return jax.lax.dot_general(a, b, (((0,), (0,)), ((), ())), preferred_element_type=f32)


def _iota(shape, dim):
    return jax.lax.broadcasted_iota(jnp.int32, shape, dim)


def _zero_after(v):
    return jnp.where(v * v < 0.0, 1.0, 0.0)


TIE = 1.1754943508222875e-38


def _relu(h):
    return jnp.where(h == 0.0, TIE, jnp.maximum(h, 0.0)).astype(bf16)


def _relu_bwd(hb, dh):
    hf = hb.astype(f32)
    return jnp.where(hf > TIE, dh, jnp.where(hf > 0.0, 0.5 * dh, 0.0)).astype(bf16)


def _pair(v, op):
    v = op(v, pltpu.roll(v, 4, v.ndim - 2))
    return op(v, pltpu.roll(v, 2, v.ndim - 2))


def _phi(p):
    p4 = p.reshape(NG, 8, 8, p.shape[-1])
    mx = _pair(jnp.max(p4, axis=1), jnp.maximum)
    mn = _pair(jnp.min(p4, axis=1), jnp.minimum)
    ep = jnp.exp(p4 - mx[:, None])
    en = jnp.exp(mn[:, None] - p4)
    sp = _pair(jnp.sum(ep, axis=1), jnp.add)
    sn = _pair(jnp.sum(en, axis=1), jnp.add)
    return ep * (1.0 / sp)[:, None], en * (1.0 / sn)[:, None]


def _softmax_bwd(ph, dph):
    t = ph.shape[-1]
    ph = ph.reshape(2, 8, 8, t)
    dph = dph.reshape(2, 8, 8, t)
    u = ph * dph
    r = _pair(jnp.sum(u, axis=1), jnp.add)
    w = u - ph * r[:, None]
    return (w[0] - w[1]).reshape(64, t)


def _kernel(x_hbm, wqkv_hbm, wphi_hbm, wo_hbm, w1_hbm, w2_hbm, do_hbm,
            out_hbm, dx_hbm, dwqkv_hbm, dwphi_hbm, dwo_hbm, dw1_hbm, dw2_hbm,
            X, DO, WQKV, WO, W1, W2, WT, PHIPT, XN, RSTD, PHIQ, PHIK, VT, Hs, DHs, F, DS, OT,
            KVT, KVTm, KVm, ZB, DNE, DXN, wphi_ref, GATE,
            xsem, wsem, isem, osem, qsem):
    XB = (0, 512, 896, 2048)

    def cp_x(i):
        return pltpu.make_async_copy(x_hbm.at[XB[i]:XB[i + 1], :], X.at[XB[i]:XB[i + 1], :], xsem.at[i])

    def cp_w1(i):
        return pltpu.make_async_copy(w1_hbm.at[:, i * CH:(i + 1) * CH], W1.at[:, i * CH:(i + 1) * CH], wsem.at[i])

    def cp_wqkv(i, part):
        cols = pl.ds(pl.multiple_of(part * D + i * 256, 256), 256)
        return pltpu.make_async_copy(wqkv_hbm.at[:, cols], WQKV.at[:, cols], qsem.at[3 * i + part])

    cp_wo = pltpu.make_async_copy(wo_hbm, WO, isem.at[1])
    cp_w2 = pltpu.make_async_copy(w2_hbm, W2, isem.at[2])
    cp_do = pltpu.make_async_copy(do_hbm, DO, isem.at[3])
    cp_wphi = pltpu.make_async_copy(wphi_hbm, wphi_ref, isem.at[4])
    dwphi_ref = wphi_ref
    cp_x(0).start()
    cp_w1(0).start()

    r128 = _iota((128, 128), 0)
    c128 = _iota((128, 128), 1)
    def head_of(r):
        return (r // 64) * 2 + r % 2

    def feat_of(r):
        return (r % 64) // 2

    rE = _iota((EXT, 128), 0)
    maskE = jnp.where(rE < 64, rE // 32, (rE - 64) // 8) == (_iota((EXT, 128), 1) % 2)

    VT[:, 64:EXT, :] = jnp.ones((NG, EXT - 64, S), bf16)
    KVT[...] = jnp.zeros_like(KVT)
    KVm[...] = jnp.zeros_like(KVm)

    def ln_fwd(r0, n, chain):
        dep = None
        for a in range(0, n, LF):
            rows = pl.ds(pl.multiple_of(r0 + a, LF), LF)
            x = X[rows, :].astype(f32)
            mu = jnp.mean(x, axis=-1, keepdims=True)
            if chain and dep is not None:
                mu = mu + _zero_after(dep)
            xc = x - mu
            var = jnp.mean(xc * xc, axis=-1, keepdims=True)
            rstd = jax.lax.rsqrt(var + 1e-5)
            dep = rstd
            XN[rows, :] = (xc * rstd).astype(bf16)
            RSTD[rows, :] = jnp.broadcast_to(rstd, (LF, 128))

    def h_mm(r0, r1, j):
        Hs[r0:r1, j * CH:(j + 1) * CH] = _relu(_nn(XN[r0:r1, :], W1[:, j * CH:(j + 1) * CH]))

    R0 = XB[1]
    RB = 384
    NRB = (S - R0) // RB
    with jax.named_scope("s1a"):
        cp_x(0).wait()
        ln_fwd(0, R0, False)
        cp_w1(0).wait()
        cp_w1(1).start()
        cp_w1(2).start()
        h_mm(0, R0, 0)
        cp_w1(1).wait()
        cp_w1(3).start()
        cp_w1(4).start()
        h_mm(0, R0, 1)
        cp_w1(2).wait()
        cp_w1(5).start()
        cp_w1(6).start()
        cp_wphi.start()
        h_mm(0, R0, 2)
        cp_w1(3).wait()
        cp_w1(4).wait()
        cp_x(1).start()
        cp_x(2).start()
        h_mm(0, R0, 3)
        h_mm(0, R0, 4)
        cp_w1(5).wait()
        cp_w1(6).wait()
        cp_x(1).wait()
        cp_wphi.wait()
        for part in range(3):
            cp_wqkv(0, part).start()
        E = jnp.where(feat_of(_iota((32, 128), 1)) == _iota((32, 128), 0), 1.0, 0.0).astype(bf16)
        rep = _nn(wphi_ref[...], E)
        phip = jnp.where((_iota((1024, 128), 0) // 32) % 4 == head_of(_iota((1024, 128), 1)), rep, 0.0)
        for g in range(NB):
            PHIPT[g] = phip[g * 128:(g + 1) * 128, :].T.astype(bf16)

        ln_fwd(R0, RB, True)
        h_mm(0, R0, 5)
        h_mm(0, R0, 6)

    def s1b_body(i, c):
        for part in range(3):
            cp_wqkv(i, part).wait()
        rows = pl.ds(pl.multiple_of(R0 + i * RB, 128), RB)
        xn = XN[rows, :]
        ln_fwd(R0 + jnp.minimum(i + 1, NRB - 1) * RB, RB, True)
        for j in range(NCH):
            Hs[rows, j * CH:(j + 1) * CH] = _relu(_nn(xn, W1[:, j * CH:(j + 1) * CH]))
            if j in (4, 5):
                g = 2 * i + (j == 5)
                c0 = pl.multiple_of(g * 128, 128)
                pt = PHIPT[g]
                WT[pl.ds(c0, 128), :] = _nt(pt, WQKV[:, pl.ds(c0, 128)]).astype(bf16)
                WT[pl.ds(D + c0, 128), :] = _nt(pt, WQKV[:, pl.ds(D + c0, 128)]).astype(bf16)
                WT[pl.ds(2 * D + c0, 128), :] = WQKV[:, pl.ds(2 * D + c0, 128)].T
        return c

    with jax.named_scope("s1b"):
        cp_x(2).wait()
        for i in range(1, 4):
            for part in range(3):
                cp_wqkv(i, part).start()
        cp_w2.start()
        cp_wo.start()
        cp_do.start()
        jax.lax.fori_loop(0, (S - R0) // RB, s1b_body, 0)
        cp_w2.wait()
        cp_wo.wait()
        cp_do.wait()

    def gate_store(f, rows, cols):
        sig = jax.nn.sigmoid(f)
        gate = f * sig
        dout = DO[rows, cols].astype(f32)
        GATE[rows, cols] = gate.astype(bf16)
        DS[rows, cols] = (dout * gate).astype(bf16)
        F[rows, cols] = (dout * (sig * (1.0 + f * (1.0 - sig)))).astype(bf16)

    def phase_a(t, c):
        ts = pl.multiple_of(t * T, T)
        rows = pl.ds(ts, T)
        xn = XN[rows, :]
        qp, qn = _phi(_nt(WT[0:D, :], xn))
        PHIQ[:, 0:64, rows] = qp.reshape(NG, 64, T).astype(bf16)
        PHIQ[:, 64:128, rows] = qn.reshape(NG, 64, T).astype(bf16)
        kp, kn = _phi(_nt(WT[D:2 * D, :], xn))
        PHIK[:, 0:64, rows] = kp.reshape(NG, 64, T).astype(bf16)
        PHIK[:, 64:128, rows] = kn.reshape(NG, 64, T).astype(bf16)
        frows = pl.ds(pl.multiple_of(t * FR, 16), FR)
        gate_store(_nn(Hs[frows, :], W2[...]), frows, slice(None))
        VT[:, 0:64, rows] = _nt(WT[2 * D:3 * D, :], xn).reshape(NG, 64, T).astype(bf16)
        for g in range(NG):
            KVT[g] += _nt(VT[g, :, rows], PHIK[g, :, rows])
        return c

    with jax.named_scope("phaseA"):
        jax.lax.fori_loop(0, NT, phase_a, 0)

    def prep(col_from_masked):
        for p in range(NB):
            ms, zs = [], []
            for e in range(2):
                g = 2 * p + e
                kvt = KVT[g]
                m = jnp.where(maskE, kvt, 0.0)
                KVTm[g] = m.astype(bf16)
                ms.append(m[0:64, :])
                if col_from_masked:
                    zs.append(m[64:65, :] + m[72:73, :])
                else:
                    zs.append(kvt[64:65, :])
            mt = jnp.concatenate(ms, axis=0).T.astype(bf16)
            KVm[p, 0:128, 0:64] = mt[:, 0:64]
            KVm[p, 128:256, 64:128] = mt[:, 64:128]
            for e in range(2):
                ZB[2 * p + e] = jnp.broadcast_to(zs[e], (128, 128)).T

    def out_copy(t):
        rows = pl.ds(pl.multiple_of(t * T, T), T)
        return pltpu.make_async_copy(X.at[rows, :], out_hbm.at[rows, :], osem.at[0])

    def dx_copy(t):
        rows = pl.ds(pl.multiple_of(t * T, T), T)
        return pltpu.make_async_copy(DO.at[rows, :], dx_hbm.at[rows, :], osem.at[1])

    DC = 128
    NDC = DFF // DC

    def dh_mm(t, c0=0, c1=NDC, dfp=None):
        rows = pl.ds(pl.multiple_of(t * T, T), T)
        cols = slice(c0 * DC, c1 * DC)
        if dfp is None:
            dfp = F[rows, :]
        dh = _nt(dfp, W2[cols, :])
        DHs[rows, cols] = _relu_bwd(Hs[rows, cols], dh)

    def phase_b_main(t, filler):
        ts = pl.multiple_of(t * T, T)
        rows = pl.ds(ts, T)
        fc = [0]

        def fill(n):
            for _ in range(n):
                filler(fc[0])
                fc[0] += 1

        fill(2)
        o_l, rden_l = [], []
        odd = (_iota((8, T), 0) % 2) == 1
        for g in range(NG):
            ne = _nn(KVTm[g], PHIQ[g, :, rows])
            rden = (1.0 / (ne[64:80] + 1e-6)).reshape(2, 1, 8, T)
            o_l.append(ne[0:64].reshape(2, 4, 8, T) * rden)
            rden_l.append(rden)
            if g % 4 == 3:
                fill(1)
        fill(2)
        doT = _nt(WO[...], DS[rows, :])
        oT = jnp.concatenate([o.reshape(64, T) for o in o_l], axis=0).astype(bf16)
        OT[:, rows] = oT
        s = _tn(oT, WO[...])
        X[rows, :] = (X[rows, :].astype(f32) + s * GATE[rows, :].astype(f32)).astype(bf16)
        out_copy(t).start()
        F[rows, :] = (F[rows, :].astype(f32) * s).astype(bf16)
        fill(2)
        for p in range(NB):
            ddens = []
            for e in range(2):
                g = 2 * p + e
                dnum = doT[g * 64:(g + 1) * 64].reshape(2, 4, 8, T) * rden_l[g]
                dd = jnp.sum(dnum * o_l[g], axis=1)
                dd = _pair(dd, jnp.add)
                dd = -(dd + pltpu.roll(dd, 1, 1))
                DNE[g, 0:64, :] = dnum.reshape(64, T).astype(bf16)
                DNE[g, 64:EXT, :] = dd.reshape(16, T).astype(bf16)
                ddens.append(jnp.where(odd, dd[1], dd[0]))
            dphi2 = _nn(KVm[p], DNE[2 * p:2 * p + 2, 0:64, :].reshape(128, T))
            for e in range(2):
                g = 2 * p + e
                phq = PHIQ[g, :, rows]
                KVT[g] += _nt(DNE[g], phq)
                zt = jnp.concatenate([ZB[g]] * (T // 128), axis=1).reshape(16, 8, T)
                dphi = dphi2[e * 128:(e + 1) * 128].reshape(16, 8, T) + zt * ddens[e][None]
                dp = _softmax_bwd(phq.astype(f32), dphi.reshape(128, T))
                PHIQ[g, 0:64, rows] = dp.astype(bf16)
            fill(2)
        fill(2)

    def phase_b(t, c):
        dfp = F[pl.ds(pl.multiple_of((t - 1) * T, T), T), :]
        phase_b_main(t, lambda i: dh_mm(t - 1, i, i + 1, dfp))
        return c

    def f_tail(i):
        if i < 8:
            cols = slice(i * 128, (i + 1) * 128)
            gate_store(_nn(Hs[NT * FR:S, :], W2[:, cols]), slice(NT * FR, S), cols)

    with jax.named_scope("prep1"):
        prep(False)
        KVT[...] = jnp.zeros_like(KVT)
        order = {0: 0, 3: 1, 6: 2, 8: 3, 12: 4, 16: 5, 20: 6, 24: 7}
        phase_b_main(0, lambda i: f_tail(order.get(i, 99)))

    with jax.named_scope("phaseB"):
        jax.lax.fori_loop(1, NT, phase_b, 0)

    with jax.named_scope("dh7"):
        prep(True)
        dh_mm(NT - 1)
        DXN[...] = jnp.zeros_like(DXN)

    def ln_bwd_rows(t, a0, n):
        dep = None
        for a in range(0, n, LB):
            rows = pl.ds(pl.multiple_of(t * T + a0 + a, LB), LB)
            dxn = DXN[pl.ds(pl.multiple_of(a0 + a, LB), LB), :]
            xn = XN[rows, :].astype(f32)
            rstd = RSTD[rows, 0:1]
            m1 = jnp.mean(dxn, axis=-1, keepdims=True)
            if dep is not None:
                m1 = m1 + _zero_after(dep)
            m2 = jnp.mean(dxn * xn, axis=-1, keepdims=True)
            r = rstd * (dxn - m1 - xn * m2)
            dep = r[:, 0:1]
            DO[rows, :] = (DO[rows, :].astype(f32) + r).astype(bf16)

    def phase_c_main(t):
        ts = pl.multiple_of(t * T, T)
        rows = pl.ds(ts, T)
        parts = []
        for p in range(NB):
            dphi2 = _nn(KVm[p], VT[2 * p:2 * p + 2, 0:64, rows].reshape(128, T))
            for e in range(2):
                g = 2 * p + e
                phk = PHIK[g, :, rows]
                zt = jnp.concatenate([ZB[g]] * (T // 128), axis=1)
                dphi = dphi2[e * 128:(e + 1) * 128] + zt
                dv = _nn(KVTm[g, 0:64, :], phk)
                dp = _softmax_bwd(phk.astype(f32), dphi)
                PHIK[g, 0:64, rows] = dp.astype(bf16)
                VT[g, 0:64, rows] = dv.astype(bf16)
            parts.append(_nt(DHs[rows, :], W1[p * 128:(p + 1) * 128, :]))
        dxn = jnp.concatenate(parts, axis=1)
        dpt = jnp.concatenate([PHIQ[:, 0:64, rows].reshape(D, T), PHIK[:, 0:64, rows].reshape(D, T),
                               VT[:, 0:64, rows].reshape(D, T)], axis=0)
        dxn += _tn(dpt, WT[...])
        return dxn

    def phase_c(t, c):
        ln_bwd_rows(jnp.maximum(t - 1, 0), 0, T)
        DXN[...] = phase_c_main(t)

        @pl.when(t > 0)
        def _():
            dx_copy(t - 1).start()
        return c

    with jax.named_scope("phaseC"):
        jax.lax.fori_loop(0, NT, phase_c, 0)

    C2 = 896
    NC2 = DFF // C2

    def mid_body(i, c):
        r0 = pl.multiple_of(i * 256, 256)
        q0 = pl.multiple_of(i * 64, 64)
        ln_bwd_rows(NT - 1, q0, 64)
        lrows = pl.ds((NT - 1) * T + q0, 64)
        pltpu.make_async_copy(DO.at[lrows, :], dx_hbm.at[lrows, :], osem.at[1]).start()
        WO[pl.ds(r0, 256), :] = _nn(OT[pl.ds(r0, 256), :], DS[...]).astype(bf16)
        pltpu.make_async_copy(WO.at[pl.ds(r0, 256), :], dwo_hbm.at[pl.ds(r0, 256), :], osem.at[3]).start()
        cs = pl.multiple_of(i * C2, 128)
        W2[pl.ds(cs, C2), :] = _tn(Hs[:, pl.ds(cs, C2)], F[...]).astype(bf16)
        pltpu.make_async_copy(W2.at[pl.ds(cs, C2), :], dw2_hbm.at[pl.ds(cs, C2), :], osem.at[2]).start()
        OT[pl.ds(r0, 256), :] = XN[:, pl.ds(r0, 256)].T
        return c

    with jax.named_scope("dw2"):
        jax.lax.fori_loop(0, NC2, mid_body, 0)

    ET = jnp.where(feat_of(_iota((128, 32), 0)) == _iota((128, 32), 1), 1.0, 0.0).astype(bf16)
    maskP = head_of(r128) == (c128 // 32)

    def wq_copy(c0):
        cols = pl.ds(c0, 128)
        return pltpu.make_async_copy(WQKV.at[:, cols], dwqkv_hbm.at[:, cols], osem.at[5])

    def fin_body(i, c):
        def g_mm(ref):
            return _nn(ref[pl.ds(i * 2, 2), 0:64, :].reshape(128, S), XN[...]).astype(bf16)

        c0 = pl.multiple_of(i * 128, 128)
        rws = pl.ds(c0, 128)

        def dw1_mm(a, b):
            W1[rws, a:b] = _nn(OT[rws, :], DHs[:, a:b]).astype(bf16)

        gq = g_mm(PHIQ)
        gk = g_mm(PHIK)
        dw1_mm(0, 1024)
        cq = pl.ds(c0, 128)
        ck = pl.ds(D + c0, 128)
        dpt = _nn(gq, WQKV[:, cq]) + _nn(gk, WQKV[:, ck])
        dpt = jnp.where(maskP, dpt, 0.0).astype(bf16)
        pt = PHIPT[i]
        WQKV[:, cq] = _tn(gq, pt).astype(bf16)
        WQKV[:, ck] = _tn(gk, pt).astype(bf16)
        WQKV[:, pl.ds(2 * D + c0, 128)] = _nt(OT[...], VT[pl.ds(i * 2, 2), 0:64, :].reshape(128, S)).astype(bf16)
        dwphi_ref[rws, :] = _tn(dpt, ET).astype(bf16)
        pltpu.make_async_copy(wphi_ref.at[rws, :], dwphi_hbm.at[rws, :], osem.at[6]).start()
        wq_copy(c0).start()
        wq_copy(D + c0).start()
        wq_copy(2 * D + c0).start()
        dw1_mm(1024, 2560)
        pltpu.make_async_copy(W1.at[rws, 0:2560], dw1_hbm.at[rws, 0:2560], osem.at[4]).start()
        dw1_mm(2560, DFF)
        pltpu.make_async_copy(W1.at[rws, 2560:DFF], dw1_hbm.at[rws, 2560:DFF], osem.at[4]).start()
        return c

    with jax.named_scope("final"):
        jax.lax.fori_loop(0, NB, fin_body, 0)

    with jax.named_scope("drain"):
        pltpu.make_async_copy(X, out_hbm, osem.at[0]).wait()
        pltpu.make_async_copy(W2, dw2_hbm, osem.at[2]).wait()
        pltpu.make_async_copy(WO, dwo_hbm, osem.at[3]).wait()
        pltpu.make_async_copy(DO, dx_hbm, osem.at[1]).wait()
        pltpu.make_async_copy(WQKV, dwqkv_hbm, osem.at[5]).wait()
        pltpu.make_async_copy(W1, dw1_hbm, osem.at[4]).wait()
        pltpu.make_async_copy(wphi_ref, dwphi_hbm, osem.at[6]).wait()


@jax.jit
def pallas_recurrent_scan__linear_kernel_hedgehog__dense_activation_relu__prompt_kernel(
    A_x: jax.Array,
    A_wqkv: jax.Array,
    A_w_phi: jax.Array,
    A_wo: jax.Array,
    B_x: jax.Array,
    B_w1: jax.Array,
    B_w2: jax.Array,
    grad_out: jax.Array,
):
    x2 = A_x.reshape(S, D)
    do2 = grad_out.reshape(S, D)
    wphi2 = A_w_phi.reshape(H * DH, DH)
    anyspec = pl.BlockSpec(memory_space=pl.ANY)
    out_shape = (
        jax.ShapeDtypeStruct((S, D), bf16),
        jax.ShapeDtypeStruct((S, D), bf16),
        jax.ShapeDtypeStruct((D, 3 * D), bf16),
        jax.ShapeDtypeStruct((H * DH, DH), bf16),
        jax.ShapeDtypeStruct((D, D), bf16),
        jax.ShapeDtypeStruct((D, DFF), bf16),
        jax.ShapeDtypeStruct((DFF, D), bf16),
    )
    scratch = [
        pltpu.VMEM((S, D), bf16),
        pltpu.VMEM((S, D), bf16),
        pltpu.VMEM((D, 3 * D), bf16),
        pltpu.VMEM((D, D), bf16),
        pltpu.VMEM((D, DFF), bf16),
        pltpu.VMEM((DFF, D), bf16),
        pltpu.VMEM((3 * D, D), bf16),
        pltpu.VMEM((NB, 128, 128), bf16),
        pltpu.VMEM((S, D), bf16),
        pltpu.VMEM((S, 128), f32),
        pltpu.VMEM((NG, 128, S), bf16),
        pltpu.VMEM((NG, 128, S), bf16),
        pltpu.VMEM((NG, EXT, S), bf16),
        pltpu.VMEM((S, DFF), bf16),
        pltpu.VMEM((S, DFF), bf16),
        pltpu.VMEM((S, D), bf16),
        pltpu.VMEM((S, D), bf16),
        pltpu.VMEM((D, S), bf16),
        pltpu.VMEM((NG, EXT, 128), f32),
        pltpu.VMEM((NG, EXT, 128), bf16),
        pltpu.VMEM((NB, 256, 128), bf16),
        pltpu.VMEM((NG, 128, 128), f32),
        pltpu.VMEM((NG, EXT, T), bf16),
        pltpu.VMEM((T, D), f32),
        pltpu.VMEM((H * DH, DH), bf16),
        pltpu.VMEM((S, D), bf16),
        pltpu.SemaphoreType.DMA((4,)),
        pltpu.SemaphoreType.DMA((NCH,)),
        pltpu.SemaphoreType.DMA((5,)),
        pltpu.SemaphoreType.DMA((7,)),
        pltpu.SemaphoreType.DMA((12,)),
    ]
    outs = pl.pallas_call(
        _kernel,
        out_shape=out_shape,
        in_specs=[anyspec] * 7,
        out_specs=(anyspec,) * 7,
        scratch_shapes=scratch,
        compiler_params=pltpu.CompilerParams(vmem_limit_bytes=127 * 2**20),
    )(x2, A_wqkv, wphi2, A_wo, B_w1, B_w2, do2)
    out, dx, dwqkv, dwphi, dwo, dw1, dw2 = outs
    return (out.reshape(1, S, D), dx.reshape(1, S, D), dwqkv, dwphi.reshape(H, DH, DH), dwo, dw1, dw2)
```
